```python
import jax
import jax.numpy as jnp

def _softmax(x, axis=-1):
    return jax.nn.softmax(x, axis=axis)

def _gelu(x):
    return jax.nn.gelu(x, approximate=True)

def _silu(x):
    return jax.nn.silu(x)

def _sigmoid(x):
    return jax.nn.sigmoid(x)

def _layernorm(x, axis=-1, eps=1e-05):
    m = jnp.mean(x, axis=axis, keepdims=True)
    v = jnp.var(x, axis=axis, keepdims=True)
    return (x - m) / jnp.sqrt(v + eps)

def _scatter_add(tgt, idx, src, axis=0):
    return tgt.at[idx].add(src)

def _segment_sum(src, seg, n):
    return jax.ops.segment_sum(src, seg, n)

class _Rng:

    def __init__(self, key):
        self._k = key

    def _next(self):
        self._k, sub = jax.random.split(self._k)
        return sub

    def normal(self, shape):
        return jax.random.normal(self._next(), shape, dtype=jnp.bfloat16)

    def randint(self, lo, hi, shape):
        return jax.random.randint(self._next(), shape, lo, hi, dtype=jnp.int32)

    def uniform(self, shape, lo=0.0, hi=1.0):
        return jax.random.uniform(self._next(), shape, jnp.bfloat16, lo, hi)

    def permutation(self, n):
        return jax.random.permutation(self._next(), n)
kernel_name = 'recurrent_scan__ssm_conv_h3__mixer_gmlp__prompt'

def setup_inputs():
    _rng = _Rng(jax.random.key(int.from_bytes(__import__("os").urandom(4), "little")))
    _w = lambda a: (lambda t: t.astype(jnp.bfloat16) if jnp.issubdtype(t.dtype, jnp.floating) else t)(jnp.asarray(a))

    def _A_setup():
        B, S, D = (1, 2048, 640)
        ks = 4
        return {'q': _w((lambda *s: _rng.normal(s) * 0.05)(B, S, D)), 'k': _w((lambda *s: _rng.normal(s) * 0.05)(B, S, D)), 'v': _w((lambda *s: _rng.normal(s) * 0.05)(B, S, D)), 'shift_k': _w((lambda *s: _rng.normal(s) * 0.05)(D, ks) * 0.5), 'ssm_k': _w((lambda *s: _rng.normal(s) * 0.05)(D, S) * (1.0 / S ** 0.5)), 'ssm_D': _w((lambda *s: _rng.normal(s) * 0.05)(D))}
    _A_in = _A_setup()

    def _B_setup():
        B, S, D, F = (1, 2048, 640, 1536)
        Fh = F // 2
        return {'x': _w((lambda *s: _rng.normal(s) * 0.05)(B, S, D)), 'w_in': _w((lambda *s: _rng.normal(s) * 0.05)(D, 2 * Fh)), 'w_sp': _w(0.01 * (lambda *s: _rng.normal(s) * 0.05)(S, S)), 'b_sp': _w(1.0 + 0.01 * (lambda *s: _rng.normal(s) * 0.05)(S)), 'w_out': _w((lambda *s: _rng.normal(s) * 0.05)(Fh, D))}
    _B_in = _B_setup()
    return {'A_q': _A_in['q'], 'A_k': _A_in['k'], 'A_v': _A_in['v'], 'A_shift_k': _A_in['shift_k'], 'A_ssm_k': _A_in['ssm_k'], 'A_ssm_D': _A_in['ssm_D'], 'B_x': _B_in['x'], 'B_w_in': _B_in['w_in'], 'B_w_sp': _B_in['w_sp'], 'B_b_sp': _B_in['b_sp'], 'B_w_out': _B_in['w_out']}

def reference(A_q, A_k, A_v, A_shift_k, A_ssm_k, A_ssm_D, B_x, B_w_in, B_w_sp, B_b_sp, B_w_out):

    def _A_ref(q, k, v, shift_k, ssm_k, ssm_D):
        B, S, D = q.shape
        ks = shift_k.shape[-1]
        k_pad = jnp.pad(k, ((0, 0), (ks - 1, 0), (0, 0)))
        k_shift = jnp.zeros_like(k)
        for t in range(ks):
            k_shift = k_shift + k_pad[:, t:t + S, :] * shift_k[:, ks - 1 - t][None, None, :]
        kv = k_shift * v
        L = 2 * S
        kv_pad = jnp.pad(kv, ((0, 0), (0, S), (0, 0)))
        kf_pad = jnp.pad(ssm_k, ((0, 0), (0, S)))
        kv_f = (lambda x, axes=(-2, -1): jnp.fft.rfft2(x.astype(jnp.float32), axes=axes))(kv_pad[:, None, :, :], axes=(1, 2))
        kf_f = (lambda x, axes=(-2, -1): jnp.fft.rfft2(x.astype(jnp.float32), axes=axes))(kf_pad[:, None, :], axes=(1, 2))
        kf_f = (lambda x, *d: x.transpose(*d))(kf_f, 1, 2, 0)
        y_f = kv_f * kf_f[None, :, :, :]
        y = (lambda x, s, axes=(-2, -1): jnp.fft.irfft2(x, s=s, axes=axes).astype(jnp.bfloat16))(y_f, (1, L), axes=(1, 2))[:, 0, :S, :]
        y = y + kv * ssm_D[None, None, :]
        return q * y

    def _B_ref(x, w_in, w_sp, b_sp, w_out):
        B, S, D = x.shape
        F = w_in.shape[-1]
        Fh = F // 2
        z = _gelu(jnp.einsum('bsd,df->bsf', x, w_in))
        z1 = z[..., :Fh].copy()
        z2 = _layernorm(z[..., Fh:], axis=-1)
        g = jnp.einsum('ts,bsf->btf', w_sp, z2) + b_sp[None, :, None]
        return jnp.einsum('bsf,fd->bsd', z1 * g, w_out)
    x = A_q
    xn = _layernorm(x, axis=-1)
    s = _A_ref(xn, A_k, A_v, A_shift_k, A_ssm_k, A_ssm_D)
    g = _silu(_B_ref(xn, B_w_in, B_w_sp, B_b_sp, B_w_out))
    return x + s * g
```

```python
import functools
import numpy as np
import jax
import jax.numpy as jnp
from jax import lax
import jax.experimental.pallas as pl
import jax.experimental.pallas.tpu as pltpu

N1, N2 = 64, 32
N = N1 * N2
RB = 256


def _dft_tables():
    n1 = np.arange(N1)
    k1 = np.arange(N1)
    a1 = 2 * np.pi * np.outer(k1 - 0.25, n1) / N1
    f1 = np.zeros((2, 2, N1 // 2, 2, N1, 2))
    fi = np.zeros((N1, 2, N1 // 2, 2, 2, 2))
    for i in range(2):
        for j in range(2):
            f1[i, j, :, 0, :, j] = np.cos(a1[i::2])
            f1[i, j, :, 1, :, j] = -np.sin(a1[i::2])
            fi[:, j, :, i, j, 0] = np.cos(a1[i::2]).T / N
            fi[:, j, :, i, j, 1] = -np.sin(a1[i::2]).T / N
    g = np.zeros((N1 // 2, 2, 2, N2, N2 // 2, 2, 2, 2))
    gi = np.zeros((N1 // 2, 2, 2, N2 // 2, 2, 2, 2, N2))
    k2 = np.arange(N2)
    m = np.arange(N2 // 2)
    p = np.arange(N1 // 2)
    for i in range(2):
        for j in range(2):
            th = 2 * np.pi * ((2 * p + i - 0.25)[:, None, None] + N1 * k2[None, :, None]) * (2 * m + j)[None, None, :] / N
            c, s = np.cos(th), np.sin(th)
            g[:, 0, i, :, :, i, j, 0] = c
            g[:, 0, i, :, :, i, j, 1] = s
            g[:, 1, i, :, :, i, j, 0] = -s
            g[:, 1, i, :, :, i, j, 1] = c
            ct, st = c.transpose(0, 2, 1), s.transpose(0, 2, 1)
            gi[:, i, j, :, 0, 0, i, :] = ct
            gi[:, i, j, :, 0, 1, i, :] = -st
            gi[:, i, j, :, 1, 0, i, :] = st
            gi[:, i, j, :, 1, 1, i, :] = ct
    bf = lambda a, *sh: a.reshape(sh).astype(np.float32).astype(jnp.bfloat16)
    return bf(f1, 256, 128), bf(fi, 128, 256), bf(g, 32, 128, 128), bf(gi, 32, 128, 128)


_F1, _FI, _G, _GI = _dft_tables()
f32, bf16, u32 = jnp.float32, jnp.bfloat16, jnp.uint32


def _dot(a, b):
    return jnp.dot(a, b, preferred_element_type=f32)


def _ld(ref, rows):
    return jnp.concatenate([ref[t, rows, :] for t in range(ref.shape[0])], axis=1)


def _st(ref, rows, val):
    for t in range(ref.shape[0]):
        ref[t, rows, :] = val[:, t * 128:(t + 1) * 128]


def _ln(x):
    m = jnp.mean(x, axis=-1, keepdims=True)
    c = x - m
    v = jnp.mean(c * c, axis=-1, keepdims=True)
    return c * lax.rsqrt(v + 1e-5)


def _kernel(q_hbm, k_hbm, v_hbm, sk_ref, ssm_hbm, d_ref, win_hbm, wsp_hbm, b_ref, wout_hbm,
            f1_hbm, fi_hbm, g_hbm, gi_hbm, o_hbm,
            q_v, k_v, v_v, ssm_v, win_v, wsp_v, wout_v, f1_v, fi_v, g_v, gi_v,
            xn_v, z1_v, z2_v, kv_v, kt_v, ax_v, ak_v, c_v, y_v, o_v, sems, osem, *, skip=()):
    S, D = q_v.shape
    FH = z1_v.shape[1]
    NB = S // RB

    def rows(i):
        return pl.ds(i * RB, RB)

    cp_q = [pltpu.make_async_copy(q_hbm.at[rows(i)], q_v.at[rows(i)], sems.at[i]) for i in range(NB)]
    cp_k = [pltpu.make_async_copy(k_hbm.at[rows(i)], k_v.at[pl.ds(16 + i * RB, RB)], sems.at[NB + i]) for i in range(NB)]
    cp_v = [pltpu.make_async_copy(v_hbm.at[rows(i)], v_v.at[rows(i)], sems.at[2 * NB + i]) for i in range(NB)]
    cp_s = [pltpu.make_async_copy(ssm_hbm.at[:, rows(i)], ssm_v.at[:, rows(i)], sems.at[3 * NB + i]) for i in range(NB)]
    cp_w = [pltpu.make_async_copy(wsp_hbm.at[rows(i)], wsp_v.at[rows(i)], sems.at[4 * NB + i]) for i in range(NB)]
    base = 5 * NB
    cp_win = pltpu.make_async_copy(win_hbm, win_v, sems.at[base])
    cp_wout = pltpu.make_async_copy(wout_hbm, wout_v, sems.at[base + 1])
    cp_f1 = pltpu.make_async_copy(f1_hbm, f1_v, sems.at[base + 2])
    cp_fi = pltpu.make_async_copy(fi_hbm, fi_v, sems.at[base + 3])
    cp_g = pltpu.make_async_copy(g_hbm, g_v, sems.at[base + 4])
    cp_gi = pltpu.make_async_copy(gi_hbm, gi_v, sems.at[base + 5])

    cp_q[0].start(); cp_win.start(); cp_k[0].start(); cp_v[0].start(); cp_s[0].start()
    for i in range(1, NB):
        cp_q[i].start(); cp_k[i].start(); cp_v[i].start(); cp_s[i].start()
    cp_f1.start(); cp_g.start(); cp_gi.start(); cp_fi.start()
    for i in range(NB):
        cp_w[i].start()
    cp_wout.start()

    k_v[pl.ds(0, 16), :] = jnp.zeros((16, D), bf16)
    skt = jnp.transpose(jnp.pad(sk_ref[...].astype(f32), ((0, 0), (0, 124))))
    taps = [skt[s:s + 1, :] for s in range(4)]
    cp_win.wait()

    def wait_blk(cps, i):
        for t, c in enumerate(cps):
            pl.when(i == t)(c.wait)

    def phase1(i, _):
        r0 = pl.multiple_of(i * RB, RB)
        rs = pl.ds(r0, RB)
        wait_blk(cp_q, i)
        xn = _ln(q_v[rs, :].astype(f32)).astype(bf16)
        xn_v[rs, :] = xn
        z = jax.nn.gelu(_dot(xn, win_v[...]), approximate=True)
        z1_v[rs, :] = z[:, :FH].astype(bf16)
        z2_v[rs, :] = _ln(z[:, FH:]).astype(bf16)
        wait_blk(cp_k, i); wait_blk(cp_v, i); wait_blk(cp_s, i)
        ext = k_v[pl.ds(r0, RB + 16), :].astype(f32)
        ksh = ext[16:16 + RB] * taps[0]
        for s in range(1, 4):
            ksh = ksh + ext[16 - s:16 - s + RB] * taps[s]
        kv = (ksh * v_v[rs, :].astype(f32)).astype(bf16)
        hs = pl.ds(pl.multiple_of(i * (RB // 2), RB // 2), RB // 2)
        _st(kv_v, hs, pltpu.bitcast(kv, u32))
        kt = jnp.transpose(ssm_v[:, rs].astype(f32)).astype(bf16)
        _st(kt_v, hs, pltpu.bitcast(kt, u32))
        return 0

    if 'phase1' not in skip:
        lax.fori_loop(0, NB, phase1, 0)

    cp_f1.wait(); cp_g.wait(); cp_gi.wait(); cp_fi.wait()

    def fft1(m, _):
        dst = pl.ds(pl.multiple_of(m * 128, 128), 128)
        for src, out in ((kv_v, ax_v), (kt_v, ak_v)):
            t = pltpu.bitcast(_ld(src, pl.ds(m, N1, stride=16)), bf16)
            _st(out, dst, pltpu.bitcast(_dot(f1_v[...], t).astype(bf16), u32))
        return 0

    if 'fft1' not in skip:
        lax.fori_loop(0, N2 // 2, fft1, 0)

    def fft2(p, _):
        g = g_v[p]
        xh = _dot(g, pltpu.bitcast(_ld(ax_v, pl.ds(p, 64, stride=32)), bf16))
        kh = _dot(g, pltpu.bitcast(_ld(ak_v, pl.ds(p, 64, stride=32)), bf16))
        xr, xi, kr, ki = xh[:64], xh[64:], kh[:64], kh[64:]
        yh = jnp.concatenate([xr * kr - xi * ki, xr * ki + xi * kr], axis=0).astype(bf16)
        _st(c_v, pl.ds(pl.multiple_of(p * 64, 64), 64), pltpu.bitcast(_dot(gi_v[p], yh).astype(bf16), u32))
        return 0

    if 'fft2' not in skip:
        lax.fori_loop(0, N1 // 2, fft2, 0)

    def fft3(m, _):
        t = pltpu.bitcast(_ld(c_v, pl.ds(m, 128, stride=16)), bf16)
        _st(y_v, pl.ds(m, N1, stride=16), pltpu.bitcast(_dot(fi_v[...], t).astype(bf16), u32))
        return 0

    if 'fft3' not in skip:
        lax.fori_loop(0, N2 // 2, fft3, 0)

    cp_wout.wait()
    dvec = d_ref[...].astype(f32)

    def out_copy(i):
        return pltpu.make_async_copy(o_v.at[rows(i)], o_hbm.at[rows(i)], osem.at[i])

    def phase2(i, _):
        r0 = pl.multiple_of(i * RB, RB)
        rs = pl.ds(r0, RB)
        hs = pl.ds(pl.multiple_of(i * (RB // 2), RB // 2), RB // 2)
        wait_blk(cp_w, i)
        bcol = jnp.transpose(jnp.broadcast_to(b_ref[:, rs].astype(f32), (128, RB)))
        g = _dot(wsp_v[rs, :], z2_v[...]) + jnp.concatenate([bcol] * (FH // 128), axis=1)
        u = (z1_v[rs, :].astype(f32) * g).astype(bf16)
        gate = jax.nn.silu(_dot(u, wout_v[...]))
        y = pltpu.bitcast(_ld(y_v, hs), bf16).astype(f32) + pltpu.bitcast(_ld(kv_v, hs), bf16).astype(f32) * dvec
        o_v[rs, :] = (q_v[rs, :].astype(f32) + xn_v[rs, :].astype(f32) * y * gate).astype(bf16)
        for t in range(NB):
            pl.when(i == t)(out_copy(t).start)
        return 0

    if 'phase2' not in skip:
        lax.fori_loop(0, NB, phase2, 0)
    for t in range(NB):
        out_copy(t).wait()


def _impl(A_q, A_k, A_v, A_shift_k, A_ssm_k, A_ssm_D, B_x, B_w_in, B_w_sp, B_b_sp, B_w_out, **kw):
    _, S, D = A_q.shape
    F = B_w_in.shape[1]
    FH = F // 2
    NB = S // RB
    hbm = pl.BlockSpec(memory_space=pl.ANY)
    vm = pl.BlockSpec(memory_space=pltpu.VMEM)
    V = pltpu.VMEM
    out = pl.pallas_call(
        functools.partial(_kernel, **kw),
        out_shape=jax.ShapeDtypeStruct((S, D), bf16),
        in_specs=[hbm, hbm, hbm, vm, hbm, vm, hbm, hbm, vm, hbm, hbm, hbm, hbm, hbm],
        out_specs=hbm,
        scratch_shapes=[
            V((S, D), bf16), V((S + 16, D), bf16), V((S, D), bf16), V((D, S), bf16), V((D, F), bf16),
            V((S, S), bf16), V((FH, D), bf16), V((256, 128), bf16), V((128, 256), bf16),
            V((32, 128, 128), bf16), V((32, 128, 128), bf16),
            V((S, D), bf16), V((S, FH), bf16), V((S, FH), bf16), V((5, S // 2, 128), u32), V((5, S // 2, 128), u32),
            V((5, S, 128), u32), V((5, S, 128), u32), V((5, S, 128), u32), V((5, S // 2, 128), u32), V((S, D), bf16),
            pltpu.SemaphoreType.DMA((5 * NB + 6,)), pltpu.SemaphoreType.DMA((NB,)),
        ],
        compiler_params=pltpu.CompilerParams(vmem_limit_bytes=110 * 1024 * 1024),
    )(A_q.reshape(S, D), A_k.reshape(S, D), A_v.reshape(S, D), A_shift_k, A_ssm_k, A_ssm_D.reshape(1, D),
      B_w_in, B_w_sp, B_b_sp.reshape(1, S), B_w_out, _F1, _FI, _G, _GI)
    return out.reshape(1, S, D)


@jax.jit
def pallas_recurrent_scan__ssm_conv_h3__mixer_gmlp__prompt_kernel(
        A_q, A_k, A_v, A_shift_k, A_ssm_k, A_ssm_D, B_x, B_w_in, B_w_sp, B_b_sp, B_w_out):
    return _impl(A_q, A_k, A_v, A_shift_k, A_ssm_k, A_ssm_D, B_x, B_w_in, B_w_sp, B_b_sp, B_w_out)
```

```python
import functools
import numpy as np
import jax
import jax.numpy as jnp
from jax import lax
import jax.experimental.pallas as pl
import jax.experimental.pallas.tpu as pltpu

N1, N2 = 64, 32
N = N1 * N2
RB = 256


def _dft_tables():
    n1 = np.arange(N1)
    k1 = np.arange(N1)
    a1 = 2 * np.pi * np.outer(k1 - 0.25, n1) / N1
    f1 = np.zeros((2, 2, 2, N1 // 2, N1, 2))
    fi = np.zeros((2, N1, N1 // 2, 2, 2, 2))
    for i in range(2):
        for j in range(2):
            f1[0, i, j, :, :, j] = np.cos(a1[i::2])
            f1[1, i, j, :, :, j] = -np.sin(a1[i::2])
            fi[j, :, :, i, j, 0] = np.cos(a1[i::2]).T / N
            fi[j, :, :, i, j, 1] = -np.sin(a1[i::2]).T / N
    u, b, h = np.meshgrid(np.arange(16), np.arange(2), np.arange(2), indexing='ij')
    f1k = f1[..., (4 * u + b + 2 * h).ravel(), :].transpose(0, 1, 2, 3, 5, 4)
    g = np.zeros((N1 // 2, 2, 2, N2, N2 // 2, 2, 2, 2))
    gi = np.zeros((N1 // 2, 2, 2, 2, N2 // 2, 2, 2, N2))
    k2 = np.arange(N2)
    m = np.arange(N2 // 2)
    p = np.arange(N1 // 2)
    for i in range(2):
        for j in range(2):
            th = 2 * np.pi * ((2 * p + i - 0.25)[:, None, None] + N1 * k2[None, :, None]) * (2 * m + j)[None, None, :] / N
            c, s = np.cos(th), np.sin(th)
            g[:, 0, i, :, :, i, j, 0] = c
            g[:, 0, i, :, :, i, j, 1] = s
            g[:, 1, i, :, :, i, j, 0] = -s
            g[:, 1, i, :, :, i, j, 1] = c
            ct, st = c.transpose(0, 2, 1), s.transpose(0, 2, 1)
            gi[:, 0, i, j, :, 0, i, :] = ct
            gi[:, 0, i, j, :, 1, i, :] = -st
            gi[:, 1, i, j, :, 0, i, :] = st
            gi[:, 1, i, j, :, 1, i, :] = ct
    bf = lambda a, *sh: a.reshape(sh).astype(np.float32).astype(jnp.bfloat16)
    return bf(np.concatenate([f1.reshape(256, 128), f1k.reshape(256, 128)]), 2, 256, 128), bf(fi, 128, 256), bf(g, 32, 128, 128), bf(gi, 32, 128, 128)


_F1, _FI, _G, _GI = _dft_tables()
f32, bf16, u32 = jnp.float32, jnp.bfloat16, jnp.uint32


def _when(c):
    if isinstance(c, bool):
        return lambda f: f() if c else None
    return pl.when(c)


def _dot(a, b):
    return jnp.dot(a, b, preferred_element_type=f32)


def _ln(x, eps=1e-5, scale=1.0):
    m = jnp.mean(x, axis=-1, keepdims=True)
    c = x - m
    v = jnp.mean(c * c, axis=-1, keepdims=True)
    return c * (scale * lax.rsqrt(v + eps))


_GC1 = float(np.sqrt(2 / np.pi))
_GC2 = float(np.sqrt(2 / np.pi) * 0.044715)


def _gelu2(h):
    return h + h * jnp.tanh(h * (_GC1 + _GC2 * (h * h)))


def _lo(w):
    return pltpu.unpack_elementwise(w, index=0, packed_dtype=bf16, unpacked_dtype=f32)


def _hi(w):
    return pltpu.unpack_elementwise(w, index=1, packed_dtype=bf16, unpacked_dtype=f32)


def _pack(lo, hi):
    return pltpu.pack_elementwise([lo, hi], packed_dtype=bf16)


def _ld(ref, rows):
    return pltpu.bitcast(jnp.concatenate([ref[t, rows, :] for t in range(ref.shape[0])], axis=1), bf16)


def _ld_groups(ref, base, groups, n, pitch):
    return jnp.concatenate([
        jnp.concatenate([ref[t, pl.ds(base + g * pitch, n), :] for g in range(groups)], axis=0)
        for t in range(ref.shape[0])], axis=1)


def _st_groups(ref, base, groups, n, pitch, w):
    for t in range(ref.shape[0]):
        for g in range(groups):
            ref[t, pl.ds(base + g * pitch, n), :] = w[g * n:(g + 1) * n, t * 128:(t + 1) * 128]


def _kernel(q_hbm, k_hbm, v_hbm, sk_ref, ssm_hbm, d_ref, win_hbm, wsp_hbm, b_ref, wout_hbm,
            f1_hbm, fi_hbm, g_hbm, gi_hbm, o_hbm,
            q_v, v_v, ssm_v, win_v, wsp_v, wout_v, f1_v, fi_v, g_v, gi_v,
            xn_v, z1_v, z2_v, kv_v, kt_v, ax_v, ak_v, c_v, y_v, o_v, kx_v, zf_v, sems, osem, isem, *, skip=(), U1=16, U2=32, U3=16, LAG=4, LR=16, CR=16, CW=256, NS=4, SC=2, UP1=0, UP2=1):
    S, D = q_v.shape
    FH = z1_v.shape[1]
    NB = S // RB
    HB = RB // 2

    def rows(i):
        return pl.ds(pl.multiple_of(i * RB, RB), RB)

    def cp_q(i): return pltpu.make_async_copy(q_hbm.at[rows(i)], q_v.at[rows(i)], sems.at[0, i])
    class cp_k:
        def __init__(self, i):
            kw = k_hbm.bitcast(u32)
            self.c = [pltpu.make_async_copy(kw.at[pl.ds(pl.multiple_of(i * HB, HB), HB), t * 128:(t + 1) * 128],
                                            kx_v.at[t, pl.ds(pl.multiple_of(8 + i * HB, 8), HB)], sems.at[1, i]) for t in range(D // 128)]
        def start(self):
            for c in self.c: c.start()
        def wait(self):
            for c in self.c: c.wait()
    def cp_v(i): return pltpu.make_async_copy(v_hbm.at[rows(i)], v_v.at[rows(i)], sems.at[2, i])
    def cp_s(i): return pltpu.make_async_copy(ssm_hbm.at[:, rows(i)], ssm_v.at[:, rows(i)], sems.at[3, i])
    def cp_w(i): return pltpu.make_async_copy(wsp_hbm.at[rows(i)], wsp_v.at[rows(i)], sems.at[4, i])
    def cp_o(i): return pltpu.make_async_copy(o_v.at[rows(i)], o_hbm.at[rows(i)], osem.at[i])
    whole = [None] + [pltpu.make_async_copy(a, b, sems.at[5, j]) for j, (a, b) in enumerate(
        ((wout_hbm, wout_v), (f1_hbm, f1_v), (fi_hbm, fi_v), (g_hbm, g_v), (gi_hbm, gi_v)))]

    NC = 2 * FH // CW
    def cp_i(c): return pltpu.make_async_copy(win_hbm.at[:, c * CW:(c + 1) * CW], win_v.at[:, c * CW:(c + 1) * CW], isem.at[c])
    cp_q(0).start()
    for c in range(NC):
        cp_i(c).start()
    cp_k(0).start(); cp_v(0).start(); cp_s(0).start()
    cp_q(1).start()
    kx_v[:, pl.ds(0, 8), :] = jnp.zeros((D // 128, 8, 128), u32)
    sk = sk_ref[...].astype(f32)
    taps = [sk[s:s + 1, :] for s in range(4)]
    vw = v_v.bitcast(u32)

    def ln1_items(i):
        def item(j):
            r = pl.ds(pl.multiple_of(i * RB + j * LR, LR), LR)
            xn_v[r, :] = _ln(q_v[r, :].astype(f32)).astype(bf16)
        return [functools.partial(item, j) for j in range(RB // LR)]

    def ln2_items(i):
        def item(j):
            r = pl.ds(pl.multiple_of(i * RB + j * LR, LR), LR)
            z2_v[r, :] = _ln(zf_v[i % 2, pl.ds(j * LR, LR), :], 4e-5, 0.5).astype(bf16)
        return [functools.partial(item, j) for j in range(RB // LR)]

    def conv_items(i):
        h0 = i * HB
        base = i * (HB // 16 * 17)

        def item(t, j):
            ls = slice(t * 128, (t + 1) * 128)
            w0, w1, w2 = (kx_v[t, pl.ds(h0 + j * CR + o, CR), :] for o in (8, 7, 6))
            e0, o0, e1, o1, o2 = _lo(w0), _hi(w0), _lo(w1), _hi(w1), _hi(w2)
            wv = vw[pl.ds(pl.multiple_of(h0 + j * CR, CR), CR), ls]
            tp = [x[:, ls] for x in taps]
            ke = (e0 * tp[0] + o1 * tp[1] + e1 * tp[2] + o2 * tp[3]) * _lo(wv)
            ko = (o0 * tp[0] + e0 * tp[1] + o1 * tp[2] + e1 * tp[3]) * _hi(wv)
            w = _pack(ke, ko)
            for g in range(CR // 16):
                kv_v[t, pl.ds(base + (j * (CR // 16) + g) * 17, 16), :] = w[g * 16:(g + 1) * 16]

        def kt_item(t, j):
            kt = jnp.transpose(ssm_v[t * 128:(t + 1) * 128, pl.ds(pl.multiple_of(i * RB + j * 128, 128), 128)].astype(f32))
            w = _pack(kt[:64], kt[64:])
            for g in range(2):
                kt_v[t, pl.ds((i * (RB // 64) + j * 2 + g) * 33, 32), :] = w[g * 32:(g + 1) * 32]

        out = []
        for t in range(D // 128):
            out += [functools.partial(item, t, j) for j in range(HB // CR)]
            out += [functools.partial(kt_item, t, j) for j in range(RB // 128)]
        return out

    def spread(items, n):
        return [items[len(items) * c // n:len(items) * (c + 1) // n] for c in range(n)]

    with jax.named_scope('w_q0'):
        cp_q(0).wait()
    for f in ln1_items(0):
        f()
    NC = 2 * FH // CW

    def phase1(i, _, first=False):
        rs = rows(i)
        if not first:
            @_when(i + 1 < NB)
            def _():
                cp_k(i + 1).start(); cp_v(i + 1).start(); cp_s(i + 1).start()
            _when(i + 2 < NB)(lambda: cp_q(i + 2).start())
            @_when(i == 3)
            def _():
                for c in whole[2:]:
                    c.start()
            _when(i + 1 < NB)(lambda: cp_q(i + 1).wait())
            with jax.named_scope('w_p1'):
                cp_k(i).wait(); cp_v(i).wait(); cp_s(i).wait()
        items = conv_items(i) + ln1_items(jnp.minimum(i + 1, NB - 1))[:0 if isinstance(i, int) and i == NB - 1 else None] + ([] if first else ln2_items(i - 1))
        side = spread(items, NS) + [[]] * (NC - NS)
        if first:
            side = [[]] * (NC // 2) + spread(items, NC - NC // 2)
        xn = xn_v[rs, :]
        for c in range(NC):
            z1c = c < NC // 2
            col = c * CW
            if first:
                with jax.named_scope('w_i'):
                    cp_i(c).wait()
                if c == SC:
                    cp_q(2).start(); cp_k(1).start(); cp_v(1).start(); cp_s(1).start()
                if c == NC // 2:
                    with jax.named_scope('w_kvs'):
                        cp_k(0).wait(); cp_v(0).wait(); cp_s(0).wait(); cp_q(1).wait()
            z = _dot(xn, win_v[:, col:col + CW])
            if z1c:
                z1_v[rs, col:col + CW] = z.astype(bf16)
            else:
                zf_v[i % 2, :, col - FH:col - FH + CW] = _gelu2(z)
            for f in side[c]:
                f()
        return 0

    with jax.named_scope('P1'):
        phase1(0, 0, True)
        if UP1:
            for i in range(1, NB):
                phase1(i, 0)
        else:
            lax.fori_loop(1, NB, phase1, 0)
        for j in range(NB):
            cp_w(j).start()
            if j == 0:
                whole[1].start()
        for f in ln2_items(NB - 1):
            f()

    with jax.named_scope('w_const'):
        for c in whole[2:]:
            c.wait()

    def fft1(mo, _):
        for u in range(U1):
            m = mo * U1 + u
            tx = _ld(kv_v, pl.ds(m, N1, stride=17))
            tk = jnp.concatenate([_ld(kt_v, pl.ds(2 * m + j, 32, stride=33)) for j in range(2)], axis=0)
            for f1, t, out in ((f1_v[0], tx, ax_v), (f1_v[1], tk, ak_v)):
                a = _dot(f1, t)
                _st_groups(out, m * (4 * 33), 4, 32, 33, _pack(a[:128], a[128:]))
        return 0

    if 'fft1' not in skip:
        with jax.named_scope('F1'):
            lax.fori_loop(0, N2 // 2 // U1, fft1, 0)

    def fft2(po, _):
        def fwd(p, t):
            g = g_v[p]
            xh = _dot(g, pltpu.bitcast(ax_v[t, pl.ds(p, 64, stride=33), :], bf16))
            kh = _dot(g, pltpu.bitcast(ak_v[t, pl.ds(p, 64, stride=33), :], bf16))
            xr, xi, kr, ki = xh[:64], xh[64:], kh[:64], kh[64:]
            return jnp.concatenate([xr * kr - xi * ki, xr * ki + xi * kr], axis=0).astype(bf16)

        def inv(p, t, yh):
            c = _dot(gi_v[p], yh)
            w = _pack(c[:64], c[64:])
            for g in range(4):
                c_v[t, pl.ds(p * (4 * 17) + g * 17, 16), :] = w[g * 16:(g + 1) * 16]

        units = [(po * U2 + u, t) for u in range(U2) for t in range(D // 128)]
        pend = []
        for un in units:
            pend.append(un + (fwd(*un),))
            if len(pend) > LAG:
                inv(*pend.pop(0))
        for e in pend:
            inv(*e)
        return 0

    if 'fft2' not in skip:
        with jax.named_scope('F2'):
            lax.fori_loop(0, N1 // 2 // U2, fft2, 0)

    def fft3(mo, _):
        for u in range(U3):
            m = mo * U3 + u
            y = _dot(fi_v[...], _ld(c_v, pl.ds(m, 128, stride=17)))
            y = _pack(y[:N1], y[N1:])
            for t in range(D // 128):
                y_v[t, pl.ds(m, N1, stride=17), :] = y[:, t * 128:(t + 1) * 128]
        return 0

    if 'fft3' not in skip:
        with jax.named_scope('F3'):
            lax.fori_loop(0, N2 // 2 // U3, fft3, 0)

    whole[1].wait()
    dvec = d_ref[...].astype(f32).reshape(1, D)

    def phase2(i, _):
        rs = rows(i)
        with jax.named_scope('w_w'):
            cp_w(i).wait()
        brow = 0.5 * b_ref[rs].astype(f32).reshape(1, RB)
        bcol = jnp.transpose(jnp.broadcast_to(brow, (128, RB)))
        g = _dot(wsp_v[rs, :], z2_v[...]) + jnp.concatenate([bcol] * (FH // 128), axis=1)
        u = (_gelu2(z1_v[rs, :].astype(f32)) * g).astype(bf16)
        gate = jax.nn.silu(_dot(u, wout_v[...]))
        base = i * (HB // 16 * 17)
        y = pltpu.bitcast(_ld_groups(y_v, base, HB // 16, 16, 17), bf16).astype(f32)
        kv = pltpu.bitcast(_ld_groups(kv_v, base, HB // 16, 16, 17), bf16).astype(f32)
        o_v[rs, :] = (q_v[rs, :].astype(f32) + xn_v[rs, :].astype(f32) * (y + kv * dvec) * gate).astype(bf16)
        cp_o(i).start()
        return 0

    with jax.named_scope('P2'):
        lax.fori_loop(0, NB // UP2, lambda o, _: [phase2(o * UP2 + u, 0) for u in range(UP2)][0], 0)
    with jax.named_scope('w_o'):
        for t in range(NB):
            cp_o(t).wait()


def _impl(A_q, A_k, A_v, A_shift_k, A_ssm_k, A_ssm_D, B_x, B_w_in, B_w_sp, B_b_sp, B_w_out, flags=None, **kw):
    _, S, D = A_q.shape
    F = B_w_in.shape[1]
    FH = F // 2
    NB = S // RB
    T = D // 128
    hbm = pl.BlockSpec(memory_space=pl.ANY)
    vm = pl.BlockSpec(memory_space=pltpu.VMEM)
    V = pltpu.VMEM
    out = pl.pallas_call(
        functools.partial(_kernel, **kw),
        out_shape=jax.ShapeDtypeStruct((S, D), bf16),
        in_specs=[hbm, hbm, hbm, vm, hbm, vm, hbm, hbm, vm, hbm, hbm, hbm, hbm, hbm],
        out_specs=hbm,
        scratch_shapes=[
            V((S, D), bf16), V((S, D), bf16), V((D, S), bf16), V((D, F), bf16),
            V((S, S), bf16), V((FH, D), bf16), V((2, 256, 128), bf16), V((128, 256), bf16),
            V((32, 128, 128), bf16), V((32, 128, 128), bf16),
            V((S, D), bf16), V((S, FH), bf16), V((S, FH), bf16), V((T, 64 * 17, 128), u32), V((T, 32 * 33, 128), u32),
            V((T, 64 * 33, 128), u32), V((T, 64 * 33, 128), u32), V((T, 128 * 17, 128), u32), V((T, 64 * 17, 128), u32),
            V((S, D), bf16), V((T, S // 2 + 8, 128), u32), V((2, RB, FH), f32),
            pltpu.SemaphoreType.DMA((6, NB)), pltpu.SemaphoreType.DMA((NB,)), pltpu.SemaphoreType.DMA((12,)),
        ],
        compiler_params=pltpu.CompilerParams(vmem_limit_bytes=110 * 1024 * 1024, flags=flags),
    )(A_q.reshape(S, D), A_k.reshape(S, D), A_v.reshape(S, D), A_shift_k.T, A_ssm_k, A_ssm_D,
      B_w_in, B_w_sp, B_b_sp, B_w_out, _F1, _FI, _G, _GI)
    return out.reshape(1, S, D)


@jax.jit
def pallas_recurrent_scan__ssm_conv_h3__mixer_gmlp__prompt_kernel(
        A_q, A_k, A_v, A_shift_k, A_ssm_k, A_ssm_D, B_x, B_w_in, B_w_sp, B_b_sp, B_w_out):
    return _impl(A_q, A_k, A_v, A_shift_k, A_ssm_k, A_ssm_D, B_x, B_w_in, B_w_sp, B_b_sp, B_w_out)
```
